```python
import os as _os
_os.environ.setdefault("JAX_PLATFORMS", "cpu")
import jax
import jax.numpy as jnp

def _softmax(x, axis=-1):
    return jax.nn.softmax(x, axis=axis)
def _gelu(x):
    return jax.nn.gelu(x, approximate=True)
def _silu(x):
    return jax.nn.silu(x)
def _sigmoid(x):
    return jax.nn.sigmoid(x)
def _layernorm(x, axis=-1, eps=1e-5):
    m = jnp.mean(x, axis=axis, keepdims=True)
    v = jnp.var(x, axis=axis, keepdims=True)
    return (x - m) / jnp.sqrt(v + eps)
def _scatter_add(tgt, idx, src, axis=0):
    return tgt.at[idx].add(src)
def _segment_sum(src, seg, n):
    return jax.ops.segment_sum(src, seg, n)
class _Rng:
    def __init__(self, key):
        self._k = key
    def _next(self):
        self._k, sub = jax.random.split(self._k)
        return sub
    def normal(self, shape):
        return jax.random.normal(self._next(), shape, dtype=jnp.bfloat16)
    def randint(self, lo, hi, shape):
        return jax.random.randint(self._next(), shape, lo, hi, dtype=jnp.int32)
    def uniform(self, shape, lo=0.0, hi=1.0):
        return jax.random.uniform(self._next(), shape, jnp.bfloat16, lo, hi)
    def permutation(self, n):
        return jax.random.permutation(self._next(), n)


kernel_name = 'recurrent_scan__ssm_conv_s4__mixer_s_mlp__prompt'

def setup_inputs():
    _rng = _Rng(jax.random.key(int.from_bytes(__import__("os").urandom(4), "little")))
    _w = (lambda a: (lambda t: t.astype(jnp.bfloat16) if jnp.issubdtype(t.dtype, jnp.floating) else t)(jnp.asarray(a)))
    def _A_setup():
        B, L, D, N = 1, 2048, 512, 128
        A_re = -jnp.exp((lambda *s: _rng.normal(s) * 0.1)(D, N))
        A_im = jnp.pi * (lambda *s: _rng.normal(s) * 0.1)(D, N)
        B_re = (lambda *s: _rng.normal(s) * 0.1)(D, N)
        B_im = (lambda *s: _rng.normal(s) * 0.1)(D, N)
        C_re = (lambda *s: _rng.normal(s) * 0.1)(D, N)
        C_im = (lambda *s: _rng.normal(s) * 0.1)(D, N)
        log_dt = (lambda *s: _rng.normal(s) * 0.1)(D) * 0.5 - 4.0
        Dskip = (lambda *s: _rng.normal(s) * 0.05)(D)
        return {
            "u": _w((lambda *s: _rng.normal(s) * 0.05)(B, L, D)),
            "A_re": _w(A_re),
            "A_im": _w(A_im),
            "B_re": _w(B_re),
            "B_im": _w(B_im),
            "C_re": _w(C_re),
            "C_im": _w(C_im),
            "log_dt": _w(log_dt),
            "Dskip": _w(Dskip),
        }
    _A_in = _A_setup()

    def _B_setup():
        B, S, D, F = 1, 2048, 512, 1376
        return {
            "x":  _w((lambda *s: _rng.normal(s) * 0.05)(B, S, D)),
            "w1": _w((lambda *s: _rng.normal(s) * 0.8)(D, D) * (D ** -0.5)),
            "w2": _w((lambda *s: _rng.normal(s) * 0.8)(D, D) * (D ** -0.5)),
            "w3": _w((lambda *s: _rng.normal(s) * 0.8)(D, F) * (D ** -0.5)),
            "w4": _w((lambda *s: _rng.normal(s) * 0.8)(F, D) * (F ** -0.5)),
        }
    _B_in = _B_setup()

    return {
        "A_u": _A_in["u"],
        "A_A_re": _A_in["A_re"],
        "A_A_im": _A_in["A_im"],
        "A_B_re": _A_in["B_re"],
        "A_B_im": _A_in["B_im"],
        "A_C_re": _A_in["C_re"],
        "A_C_im": _A_in["C_im"],
        "A_log_dt": _A_in["log_dt"],
        "A_Dskip": _A_in["Dskip"],
        "B_x": _B_in["x"],
        "B_w1": _B_in["w1"],
        "B_w2": _B_in["w2"],
        "B_w3": _B_in["w3"],
        "B_w4": _B_in["w4"],
    }

def reference(A_u, A_A_re, A_A_im, A_B_re, A_B_im, A_C_re, A_C_im, A_log_dt, A_Dskip, B_x, B_w1, B_w2, B_w3, B_w4):
    def _A_ref(u, A_re, A_im, B_re, B_im, C_re, C_im, log_dt, Dskip):
        Bsz, L, D = u.shape
        dt = jnp.exp(log_dt)[:, None]
        A = A_re + 1j * A_im
        Bc = B_re + 1j * B_im
        Cc = C_re + 1j * C_im
        logdA = dt * A
        dB = dt * Bc
        l = (lambda x, dt: x.astype(dt))(jnp.arange(L), A_re.dtype)
        P = jnp.exp(logdA[:, :, None] * l[None, None, :])
        K = jnp.einsum("dn,dnl,dn->dl", Cc, P, dB).real
        L2 = 2 * L
        Kp = jnp.pad(K, ((0, 0), (0, L)))
        up = (lambda x, *d: x.transpose(*d))(u, 0, 2, 1)
        up = jnp.pad(up, ((0, 0), (0, 0), (0, L)))
        Kf = (lambda x, axes=(-2,-1): jnp.fft.rfft2(x.astype(jnp.float32), axes=axes))(Kp[:, None, :], axes=(-2, -1))
        Uf = (lambda x, axes=(-2,-1): jnp.fft.rfft2(x.astype(jnp.float32), axes=axes))(up[:, :, None, :], axes=(-2, -1))
        Yf = Uf * Kf[None, :, :, :]
        y = (lambda x, s, axes=(-2,-1): jnp.fft.irfft2(x, s=s, axes=axes).astype(jnp.bfloat16))(Yf, (1, L2), axes=(-2, -1))[:, :, 0, :L]
        y = (lambda x, *d: x.transpose(*d))(y, 0, 2, 1) + u * Dskip[None, None, :]
        return y

    def _B_ref(x, w1, w2, w3, w4):
        B, S, D = x.shape
        h = _gelu(_layernorm(x, axis=-1) @ w1)
        c = D // 4
        g0 = jnp.pad(h[:, :, 0*c:1*c], ((0, 0), (1, 0), (0, 0)))[:, :S, :]
        g1 = jnp.pad(h[:, :, 1*c:2*c], ((0, 0), (0, 1), (0, 0)))[:, 1:, :]
        g2 = jnp.pad(h[:, :, 2*c:3*c], ((0, 0), (2, 0), (0, 0)))[:, :S, :]
        g3 = jnp.pad(h[:, :, 3*c:   ], ((0, 0), (0, 2), (0, 0)))[:, 2:, :]
        hs = jnp.concatenate([g0, g1, g2, g3], axis=-1) @ w2
        x1 = x + hs
        h2 = _gelu(_layernorm(x1, axis=-1) @ w3) @ w4
        return x1 + h2

    x = A_u
    xn = _layernorm(x, axis=-1)
    s = _A_ref(xn, A_A_re, A_A_im, A_B_re, A_B_im, A_C_re, A_C_im, A_log_dt, A_Dskip)
    g = _silu(_B_ref(xn, B_w1, B_w2, B_w3, B_w4))
    return x + s * g
```

```python
import numpy as np
import jax
import jax.numpy as jnp
from jax import lax
import jax.experimental.pallas as pl
import jax.experimental.pallas.tpu as pltpu

L = 2048
D = 512
NS = 128
C = 128
NB = L // C
FF = 1376
FP = 1376
EPS = 1e-5
CWIDTH = 384
BF = jnp.bfloat16
F32 = jnp.float32


def _bases():
    b = []
    for h in (0, 1):
        b += [(h, r) for r in range(8)]
    for h in (2, 3):
        b += [(h, r) for r in (0, 2, 4, 6)]
    for h in (4, 5, 6, 7):
        b += [(h, r) for r in (0, 4)]
    for h in range(8, 16):
        b += [(h, 0)]
    b += [(16, 0)]
    return b


BASES = _bases()
NBASE = len(BASES)
NBP = 42
NT = (NBASE + 7) // 8


def _make_tables():
    lr = np.arange(L).astype(jnp.bfloat16).astype(np.int64)
    pos = {}
    for bi, (h, r) in enumerate(BASES):
        j, bp = divmod(bi, 8)
        for lo in range(16):
            if bi == NBASE - 1 and lo > 0:
                continue
            pos.setdefault(128 * h + r + 8 * lo, (j, lo * 8 + bp))
    th = np.pi * (2 * np.arange(C) + 1) / (2 * C)
    t = np.arange(C)
    fwd = np.concatenate([np.cos(th[:, None] * t[None, :]),
                          -np.sin(th[:, None] * t[None, :])], 0)
    inv = np.concatenate([np.cos(th[None, :] * t[:, None]),
                          -np.sin(th[None, :] * t[:, None])], 1) / C
    fe = {}
    for k in range(NB):
        for m in range(C):
            l = k * C + m
            jt, lane = pos[int(lr[l])]
            a = fe.setdefault((k, jt), np.zeros((2 * C, C)))
            a[:C, lane] += np.cos(th * m)
            a[C:, lane] += -np.sin(th * m)
    keys = sorted(fe.keys())
    return (fwd.astype(np.float32), inv.astype(np.float32), keys,
            np.stack([fe[k] for k in keys]).astype(np.float32))


_FWD, _INV, FE_KEYS, _FE = _make_tables()
NFE = len(FE_KEYS)


def _layernorm(x):
    m = jnp.mean(x, axis=-1, keepdims=True)
    xc = x - m
    v = jnp.mean(xc * xc, axis=-1, keepdims=True)
    return (xc * lax.rsqrt(v + EPS)).astype(BF)


def _gelu(x):
    c0 = np.float32(np.sqrt(2.0 / np.pi))
    c1 = np.float32(np.sqrt(2.0 / np.pi) * 0.044715)
    hx = 0.5 * x
    return hx + hx * jnp.tanh(x * (c0 + c1 * (x * x)))


def _cos_sin(x):
    k = jnp.round(x * np.float32(2.0 / np.pi))
    r = x - k * np.float32(1.5703125)
    r = r - k * np.float32(4.837512969970703125e-4)
    r = r - k * np.float32(7.54978995489188216e-8)
    r2 = r * r
    sn = r + r * r2 * (np.float32(-1.6666654611e-1) + r2 * (np.float32(8.3321608736e-3)
                                                            + r2 * np.float32(-1.9515295891e-4)))
    cs = 1.0 - 0.5 * r2 + r2 * r2 * (np.float32(4.166664568298827e-2) + r2 * (
        np.float32(-1.388731625493765e-3) + r2 * np.float32(2.443315711809948e-5)))
    q = k.astype(jnp.int32)
    swap = (q & 1) != 0
    c = jnp.where(swap, sn, cs)
    s_ = jnp.where(swap, cs, sn)
    c = jnp.where(((q + 1) & 2) != 0, -c, c)
    s_ = jnp.where((q & 2) != 0, -s_, s_)
    return c, s_


def _cmul(a, b):
    return (a[0] * b[0] - a[1] * b[1], a[0] * b[1] + a[1] * b[0])


def _dot(a, b):
    return jnp.dot(a, b, preferred_element_type=F32)


def _kernel(x_hbm, are_h, aim_h, bre_h, bim_h, cre_h, cim_h, logdt, dskip,
            w1_hbm, w2_hbm, w3_hbm, w4_hbm, fwd_h, inv_h, fe_hbm,
            out_hbm,
            par_v, fwd, inv, psems,
            x_v, w1_v, w2_v, w3_v, w4_v, fe_v, xn_v, h_v, uh_v, kh_v, e_v,
            kmat_v, kt_v, out_v, yh_v, ln1_v, h2_v, sems, osems, xsems):
    cx = [pltpu.make_async_copy(x_hbm.at[pl.ds(i * 256, 256), :], x_v.at[pl.ds(i * 256, 256), :],
                                xsems.at[i]) for i in range(8)]
    c1 = pltpu.make_async_copy(w1_hbm, w1_v, sems.at[1])
    cfe = pltpu.make_async_copy(fe_hbm, fe_v, sems.at[2])
    c2 = pltpu.make_async_copy(w2_hbm, w2_v, sems.at[3])
    c3 = pltpu.make_async_copy(w3_hbm, w3_v, sems.at[4])
    c4 = pltpu.make_async_copy(w4_hbm, w4_v, sems.at[5])
    cp = [pltpu.make_async_copy(h_, par_v.at[i], psems.at[i])
          for i, h_ in enumerate((bre_h, bim_h, cre_h, cim_h))]
    ca = [pltpu.make_async_copy(h_, par_v.at[4 + i], psems.at[6 + i])
          for i, h_ in enumerate((are_h, aim_h))]
    are, aim = par_v.at[4], par_v.at[5]
    cf = pltpu.make_async_copy(fwd_h, fwd, psems.at[4])
    ci = pltpu.make_async_copy(inv_h, inv, psems.at[5])
    for c in ca + cp + [cx[0], c1, cf]:
        c.start()
    bre, bim, cre, cim = (par_v.at[i] for i in range(4))

    h_v[pl.ds(0, 8), :] = jnp.zeros((8, D), F32)
    h_v[pl.ds(L + 8, 8), :] = jnp.zeros((8, D), F32)

    dt_row = jnp.exp(logdt[...].reshape(1, D).astype(F32)).astype(BF).astype(F32)
    dt = jnp.broadcast_to(dt_row, (NS, D)).T
    ca[0].wait()
    ca[1].wait()
    a_re = dt * are[...].astype(F32)
    a_im = dt * aim[...].astype(F32)
    ph = _cos_sin(a_im)
    e_v[0] = jnp.exp(a_re) * ph[0]
    e_v[1] = jnp.exp(a_re) * ph[1]
    for _ in range(3):
        ph = (ph[0] * ph[0] - ph[1] * ph[1], 2.0 * (ph[0] * ph[1]))
    mag = jnp.exp(a_re * 8.0)
    e_v[8] = mag * ph[0]
    e_v[9] = mag * ph[1]
    for pln in range(2):
        for dl in range(8):
            e_v[2 + pln, pl.ds(7 - dl, D // 8, stride=8), :] = \
                e_v[8 + pln, pl.ds(dl, D // 8, stride=8), :]
    for _ in range(4):
        ph = (ph[0] * ph[0] - ph[1] * ph[1], 2.0 * (ph[0] * ph[1]))
    mag = jnp.exp(a_re * 128.0)
    e_v[4] = mag * ph[0]
    e_v[5] = mag * ph[1]
    for c in cp:
        c.wait()
    db = (dt * bre[...].astype(F32), dt * bim[...].astype(F32))
    cdb = _cmul((cre[...].astype(F32), cim[...].astype(F32)), db)
    e_v[6] = cdb[0]
    e_v[7] = cdb[1]

    cx[0].wait()
    c1.wait()
    cf.wait()
    for c in cx[1:] + [cfe, ci, c2, c3, c4]:
        c.start()

    sub = lax.broadcasted_iota(jnp.int32, (8, 128), 0)
    lane = lax.broadcasted_iota(jnp.int32, (8, 128), 1)
    diag = (lane % 8) == (7 - sub)

    def kgen(g):
        r0 = pl.multiple_of(g * 8, 8)
        ld = lambda i: e_v[i, pl.ds(r0, 8), :]
        e1, e8, e128, cb = (ld(0), ld(1)), (ld(2), ld(3)), (ld(4), ld(5)), (ld(6), ld(7))
        one = (jnp.ones((8, 128), F32), jnp.zeros((8, 128), F32))

        def powers(e, n):
            p = [one, e]
            for i in range(2, n):
                p.append(_cmul(p[i // 2], p[i - i // 2]))
            return p
        q = powers(e8, 16)
        rr = powers(e1, 8)
        hh = [cb]
        for i in range(1, 17):
            hh.append(_cmul(hh[-1], e128))
        rows = []
        for (h, r) in BASES:
            p = hh[h] if r == 0 else _cmul(hh[h], rr[r])
            rows.append(jnp.concatenate([p[0], -p[1]], axis=1))
        rows.append(jnp.zeros((8 * (NBP - NBASE), 256), F32))
        lhs = jnp.concatenate(rows, axis=0).astype(BF)
        rhs = jnp.concatenate(
            [jnp.concatenate([qq[0], qq[1]], axis=1) for qq in q], axis=0).astype(BF)
        return lax.dot_general(lhs, rhs, (((1,), (1,)), ((), ())),
                               preferred_element_type=F32)

    def kext(g, o):
        r0 = pl.multiple_of(g * 8, 8)
        for j in range(NT):
            w = None
            for bp in range(8):
                b = 8 * j + bp
                if b >= NBASE:
                    break
                v = jnp.where(diag, o[8 * b:8 * b + 8, :], 0.0)
                if bp:
                    v = pltpu.roll(v, bp, 1)
                w = v if w is None else w + v
            w = pltpu.roll(w, 121, 1, stride=1, stride_axis=0)
            kmat_v[pl.ds(r0, 8), pl.ds(j * 128, 128)] = w

    def phase_a(it, carry):
        r0 = pl.multiple_of(it * 256, 256)
        x = x_v[pl.ds(r0, 256), :].astype(F32)
        xn = _layernorm(x)
        xn_v[pl.ds(r0, 256), :] = xn
        xn2 = _layernorm(xn.astype(F32))

        def u_piece(q):
            uh_v[2 * it + q] = _dot(fwd[...], xn[q * C:(q + 1) * C, :])

        def w1_piece(q):
            cs = pl.ds(q * 128, 128)
            h_v[pl.ds(r0 + 8, 256), cs] = _gelu(_dot(xn2, w1_v[:, cs]))

        after = {1: [lambda: u_piece(0)], 3: [lambda: u_piece(1)], 5: [lambda: w1_piece(0)]}
        os_ = {}
        for gg in range(8):
            os_[gg] = kgen(it * 8 + gg)
            if gg >= 1:
                kext(it * 8 + gg - 1, os_.pop(gg - 1))
            for f_ in after.get(gg, []):
                f_()
        kext(it * 8 + 7, os_.pop(7))
        for q in (1, 2, 3):
            w1_piece(q)

        @pl.when(it < 7)
        def _():
            rn = pl.multiple_of((it + 1) * 256, 256)
            pltpu.make_async_copy(x_hbm.at[pl.ds(rn, 256), :], x_v.at[pl.ds(rn, 256), :],
                                  xsems.at[it + 1]).wait()
        return carry

    with jax.named_scope("phase_a"):
        lax.fori_loop(0, 8, phase_a, 0)

    cfe.wait()
    for j in range(NT):
        kt_v[pl.ds(j * 128, 128), :] = kmat_v[:, pl.ds(j * 128, 128)].T.astype(BF)
    sg = jnp.where(lax.broadcasted_iota(jnp.int32, (C, D), 0) % 2 == 0, 1.0, -1.0)
    prev = None
    for k in range(NB):
        acc = None
        for i, (kk, jt) in enumerate(FE_KEYS):
            if kk != k:
                continue
            t = _dot(fe_v[i], kt_v[pl.ds(jt * 128, 128), :])
            acc = t if acc is None else acc + t
        if prev is None:
            kh_v[k] = acc
        else:
            kh_v[k, pl.ds(0, C), :] = acc[:C] - sg * prev[C:]
            kh_v[k, pl.ds(C, C), :] = acc[C:] + sg * prev[:C]
        prev = acc

    ci.wait()
    c2.wait()
    c3.wait()
    c4.wait()

    RT = 8
    NCH = (FF + 127) // 128

    def shifted_h(t0):
        parts = []
        for gi, sh in enumerate((1, -1, 2, -2)):
            w = h_v[pl.ds(t0, C + 16), pl.ds(gi * 128, 128)]
            parts.append(w[8 - sh:8 - sh + C, :])
        return jnp.concatenate(parts, axis=1).astype(BF)

    def phase_b(T, carry):
        ia = T
        ib = NB - 1 - T
        ta = pl.multiple_of(ia * C, C)
        tb = pl.multiple_of(ib * C, C)

        def conv_tile(rt, toks=None):
            off = rt * RT if isinstance(rt, int) else pl.multiple_of(rt * RT, RT)
            rs = pl.ds(off, RT)
            rsi = pl.ds(C + off, RT)
            for lp in range(D // 128):
                ls = pl.ds(lp * 128, 128)

                def prod(k, src, tok=None):
                    kr, ki = kh_v[k, rs, ls], kh_v[k, rsi, ls]
                    ur, ui = uh_v[src, rs, ls], uh_v[src, rsi, ls]
                    if tok is not None:
                        kr = jnp.where(always, kr, tok)
                    return kr * ur - ki * ui, kr * ui + ki * ur
                br, bi = prod(0, ib, None if toks is None else toks[2 * lp])
                for k in range(1, 9):
                    pr, pi_ = prod(k, ib - k)
                    br, bi = br + pr, bi + pi_
                rr_, ri_ = None, None
                car = cai = None
                for s in range(8):
                    is_a = s <= T
                    k = jnp.where(is_a, s, s + 8 - T)
                    src = jnp.where(is_a, T - s, ib - (s + 8 - T))
                    pr, pi_ = prod(k, src, toks[2 * lp + 1] if (toks is not None and s == 0) else None)
                    rr_, ri_ = (pr, pi_) if rr_ is None else (rr_ + pr, ri_ + pi_)
                    if car is None:
                        car, cai = rr_, ri_
                    else:
                        car = jnp.where(is_a, rr_, car)
                        cai = jnp.where(is_a, ri_, cai)
                yh_v[0, rs, ls] = car
                yh_v[0, rsi, ls] = cai
                yh_v[1, rs, ls] = br + (rr_ - car)
                yh_v[1, rsi, ls] = bi + (ri_ - cai)

        always = (lax.broadcasted_iota(jnp.int32, (8, 128), 1) + T) >= 0
        tiles = list(range(C // RT))
        xn = jnp.concatenate([xn_v[pl.ds(ta, C), :], xn_v[pl.ds(tb, C), :]], axis=0).astype(F32)
        hs_in = jnp.concatenate([shifted_h(ta), shifted_h(tb)], axis=0)
        hs_parts = [_dot(hs_in, w2_v[:, pl.ds(q * 128, 128)]) for q in range(4)]
        for q in range(5):
            toks = [hs_parts[(q + p) % 4][32 * p:32 * p + 8, :] for p in range(8)]
            conv_tile(tiles.pop(0), toks)
        hs = jnp.concatenate(hs_parts, axis=1)
        x1 = xn + hs
        ln1 = _layernorm(x1)
        h2 = None
        CW = CWIDTH
        nch = (FF + CW - 1) // CW
        for j in range(nch):
            w = min(CW, FF - j * CW)
            a3 = lax.dot_general(ln1, w3_v[pl.ds(j * CW, w), :], (((1,), (1,)), ((), ())),
                                 preferred_element_type=F32)
            t = _dot(_gelu(a3).astype(BF), w4_v[pl.ds(j * CW, w), :])
            h2 = t if h2 is None else h2 + t
            n_t = -(-len(tiles) // (nch - j))
            for i in range(n_t):
                lo = 128 * (i % (w // 128)) if w >= 128 else None
                if lo is not None:
                    toks = [a3[64 * p:64 * p + 8, lo:lo + 128] for p in range(4)]
                else:
                    toks = [hs_parts[p][64 * p:64 * p + 8, :] for p in range(4)]
                toks += [t[64 * p:64 * p + 8, 128 * (i % 4):128 * (i % 4) + 128] for p in range(4)]
                conv_tile(tiles.pop(0), toks)
        assert not tiles
        z = x1 + h2
        g = z * jax.nn.sigmoid(z)
        y = jnp.concatenate([_dot(inv[...], yh_v[0].astype(BF)),
                             _dot(inv[...], yh_v[1].astype(BF))], axis=0)
        s_ = y + xn * dskip[...].reshape(1, D).astype(F32)
        x = jnp.concatenate([x_v[pl.ds(ta, C), :], x_v[pl.ds(tb, C), :]], axis=0).astype(F32)
        o = (x + s_ * g).astype(BF)
        out_v[pl.ds(ta, C), :] = o[:C]
        out_v[pl.ds(tb, C), :] = o[C:]
        pltpu.make_async_copy(out_v.at[pl.ds(ta, C), :], out_hbm.at[pl.ds(ta, C), :],
                              osems.at[ia]).start()
        pltpu.make_async_copy(out_v.at[pl.ds(tb, C), :], out_hbm.at[pl.ds(tb, C), :],
                              osems.at[ib]).start()
        return carry

    with jax.named_scope("phase_b"):
        lax.fori_loop(0, NB // 2, phase_b, 0)

    for i in range(NB):
        pltpu.make_async_copy(out_v.at[pl.ds(i * C, C), :], out_hbm.at[pl.ds(i * C, C), :],
                              osems.at[i]).wait()


@jax.jit
def pallas_recurrent_scan__ssm_conv_s4__mixer_s_mlp__prompt_kernel(
    A_u: jax.Array,
    A_A_re: jax.Array,
    A_A_im: jax.Array,
    A_B_re: jax.Array,
    A_B_im: jax.Array,
    A_C_re: jax.Array,
    A_C_im: jax.Array,
    A_log_dt: jax.Array,
    A_Dskip: jax.Array,
    B_x: jax.Array,
    B_w1: jax.Array,
    B_w2: jax.Array,
    B_w3: jax.Array,
    B_w4: jax.Array,
):
    x = A_u.reshape(L, D)
    vm = pl.BlockSpec(memory_space=pltpu.VMEM)
    hbm = pl.BlockSpec(memory_space=pltpu.HBM)
    fwd = jnp.asarray(_FWD, dtype=BF)
    inv = jnp.asarray(_INV, dtype=BF)
    fe = jnp.asarray(_FE, dtype=BF)
    out = pl.pallas_call(
        _kernel,
        out_shape=jax.ShapeDtypeStruct((L, D), BF),
        in_specs=[hbm, hbm, hbm, hbm, hbm, hbm, hbm, vm, vm, hbm, hbm, hbm, hbm, hbm, hbm, hbm],
        out_specs=hbm,
        scratch_shapes=[
            pltpu.VMEM((6, D, NS), BF),
            pltpu.VMEM((2 * C, C), BF),
            pltpu.VMEM((C, 2 * C), BF),
            pltpu.SemaphoreType.DMA((8,)),
            pltpu.VMEM((L, D), BF),
            pltpu.VMEM((D, D), BF),
            pltpu.VMEM((D, D), BF),
            pltpu.VMEM((FP, D), BF),
            pltpu.VMEM((FP, D), BF),
            pltpu.VMEM((NFE, 2 * C, C), BF),
            pltpu.VMEM((L, D), BF),
            pltpu.VMEM((L + 16, D), F32),
            pltpu.VMEM((NB, 2 * C, D), F32),
            pltpu.VMEM((NB, 2 * C, D), F32),
            pltpu.VMEM((10, D, NS), F32),
            pltpu.VMEM((D, NT * 128), F32),
            pltpu.VMEM((NT * 128, D), BF),
            pltpu.VMEM((L, D), BF),
            pltpu.VMEM((2, 2 * C, D), F32),
            pltpu.VMEM((2 * C, D), BF),
            pltpu.VMEM((2 * C, D), F32),
            pltpu.SemaphoreType.DMA((6,)),
            pltpu.SemaphoreType.DMA((NB,)),
            pltpu.SemaphoreType.DMA((8,)),
        ],
        compiler_params=pltpu.CompilerParams(vmem_limit_bytes=100 * 1024 * 1024),
    )(x, A_A_re, A_A_im, A_B_re, A_B_im, A_C_re, A_C_im,
      A_log_dt, A_Dskip,
      B_w1, B_w2, B_w3.T, B_w4, fwd, inv, fe)
    return out.reshape(1, L, D)
```
